```python
import os as _os
_os.environ.setdefault("JAX_PLATFORMS", "cpu")
import jax
import jax.numpy as jnp

def _softmax(x, axis=-1):
    return jax.nn.softmax(x, axis=axis)
def _gelu(x):
    return jax.nn.gelu(x, approximate=True)
def _silu(x):
    return jax.nn.silu(x)
def _sigmoid(x):
    return jax.nn.sigmoid(x)
def _layernorm(x, axis=-1, eps=1e-5):
    m = jnp.mean(x, axis=axis, keepdims=True)
    v = jnp.var(x, axis=axis, keepdims=True)
    return (x - m) / jnp.sqrt(v + eps)
def _scatter_add(tgt, idx, src, axis=0):
    return tgt.at[idx].add(src)
def _segment_sum(src, seg, n):
    return jax.ops.segment_sum(src, seg, n)
class _Rng:
    def __init__(self, key):
        self._k = key
    def _next(self):
        self._k, sub = jax.random.split(self._k)
        return sub
    def normal(self, shape):
        return jax.random.normal(self._next(), shape, dtype=jnp.bfloat16)
    def randint(self, lo, hi, shape):
        return jax.random.randint(self._next(), shape, lo, hi, dtype=jnp.int32)
    def uniform(self, shape, lo=0.0, hi=1.0):
        return jax.random.uniform(self._next(), shape, jnp.bfloat16, lo, hi)
    def permutation(self, n):
        return jax.random.permutation(self._next(), n)


kernel_name = 'gated_mix__ssm_conv_s5__moe_arch_mod__prompt'

def setup_inputs():
    _rng = _Rng(jax.random.key(int.from_bytes(__import__("os").urandom(4), "little")))
    _w = (lambda a: (lambda t: t.astype(jnp.bfloat16) if jnp.issubdtype(t.dtype, jnp.floating) else t)(jnp.asarray(a)))
    def _A_setup():
        B, S, D = 1, 2048, 576
        P = D
        Lambda_re = -0.5 * jnp.exp((lambda *s: _rng.normal(s) * 0.4)(P))
        Lambda_im = (lambda *s: _rng.normal(s) * 0.4)(P) * 1.0
        B_re = (lambda *s: _rng.normal(s) * 0.4)(P, D) * (D ** -0.5)
        B_im = (lambda *s: _rng.normal(s) * 0.4)(P, D) * (D ** -0.5)
        C_re = (lambda *s: _rng.normal(s) * 0.4)(D, P) * (P ** -0.5)
        C_im = (lambda *s: _rng.normal(s) * 0.4)(D, P) * (P ** -0.5)
        log_dt = (lambda *s: _rng.normal(s) * 0.4)(P) * 0.3 - 2.0
        Dskip = (lambda *s: _rng.normal(s) * 0.4)(D)
        return {
            "x": _w((lambda *s: _rng.normal(s) * 0.05)(B, S, D)),
            "Lambda_re": _w(Lambda_re),
            "Lambda_im": _w(Lambda_im),
            "B_re": _w(B_re),
            "B_im": _w(B_im),
            "C_re": _w(C_re),
            "C_im": _w(C_im),
            "log_dt": _w(log_dt),
            "Dskip": _w(Dskip),
        }
    _A_in = _A_setup()

    def _B_setup():
        B, S, D, F, C = 1, 2048, 576, 4608, 2
        return {
            "x": _w((lambda *s: _rng.normal(s) * 0.05)(B, S, D)),
            "w_r": _w((lambda *s: _rng.normal(s) * 1.6)(D)),
            "w_gate": _w((lambda *s: _rng.normal(s) * 0.1)(D, F)),
            "w_up": _w((lambda *s: _rng.normal(s) * 0.1)(D, F)),
            "w_down": _w((lambda *s: _rng.normal(s) * 0.1)(F, D)),
        }
    _B_in = _B_setup()

    return {
        "A_x": _A_in["x"],
        "A_Lambda_re": _A_in["Lambda_re"],
        "A_Lambda_im": _A_in["Lambda_im"],
        "A_B_re": _A_in["B_re"],
        "A_B_im": _A_in["B_im"],
        "A_C_re": _A_in["C_re"],
        "A_C_im": _A_in["C_im"],
        "A_log_dt": _A_in["log_dt"],
        "A_Dskip": _A_in["Dskip"],
        "B_x": _B_in["x"],
        "B_w_r": _B_in["w_r"],
        "B_w_gate": _B_in["w_gate"],
        "B_w_up": _B_in["w_up"],
        "B_w_down": _B_in["w_down"],
        "gate_w": _w((lambda *s: _rng.normal(s) * 0.05)(576) * 16.0),
    }

def reference(A_x, A_Lambda_re, A_Lambda_im, A_B_re, A_B_im, A_C_re, A_C_im, A_log_dt, A_Dskip, B_x, B_w_r, B_w_gate, B_w_up, B_w_down, gate_w):
    def _A_ref(x, Lambda_re, Lambda_im, B_re, B_im, C_re, C_im, log_dt, Dskip):
        Bsz, L, H = x.shape
        Lam = Lambda_re + 1j * Lambda_im
        Bmat = B_re + 1j * B_im
        Cmat = C_re + 1j * C_im
        dt = jnp.exp(log_dt)
        Lam_bar = jnp.exp(dt * Lam)
        B_bar = ((Lam_bar - 1.0) / Lam)[:, None] * Bmat
        Bu = jnp.einsum("bld,pd->blp", x + 0j, B_bar)
        h = jnp.zeros_like(Bu[:, 0, :])
        hs = []
        for t in range(L):
            h = Lam_bar[None, :] * h + Bu[:, t, :]
            hs.append(h)
        hseq = jnp.stack(hs, 1)
        y = 2.0 * jnp.einsum("blp,dp->bld", hseq, Cmat).real + x * Dskip[None, None, :]
        return y

    def _B_ref(x, w_r, w_gate, w_up, w_down):
        B, S, D = x.shape
        C = 2
        r = x @ w_r
        idx = jnp.argsort(-r, axis=-1)[:, :C]
        idx_e = jnp.repeat(idx.reshape(B, C, 1), D, axis=2)
        x_sel = jnp.take_along_axis(x, idx_e, axis=1)
        g = _silu(x_sel @ w_gate)
        u = x_sel @ w_up
        y = (g * u) @ w_down
        r_sel = _sigmoid(jnp.take_along_axis(r, idx, axis=1))
        y = y * r_sel.reshape(B, C, 1)
        b_off = (jnp.arange(B) * S).reshape(B, 1)
        flat_idx = (idx + b_off).reshape(B * C)
        zero = (x * 0.0).reshape(B * S, D)
        upd = _scatter_add(zero, flat_idx, y.reshape(B * C, D), axis=0)
        return x + upd.reshape(B, S, D)

    x = A_x
    g = _sigmoid((x * gate_w).sum(-1, keepdims=True))
    a = _A_ref(x, A_Lambda_re, A_Lambda_im, A_B_re, A_B_im, A_C_re, A_C_im, A_log_dt, A_Dskip)
    b = _B_ref(x, B_w_r, B_w_gate, B_w_up, B_w_down)
    return g * a + (1 - g) * b
```

```python
import functools

import jax
import jax.numpy as jnp
from jax import lax
import jax.experimental.pallas as pl
import jax.experimental.pallas.tpu as pltpu

F32 = jnp.float32
BF16 = jnp.bfloat16
I32 = jnp.int32
NN = (((1,), (0,)), ((), ()))
NT = (((1,), (1,)), ((), ()))

T, D, F = 2048, 576, 4608
LANES, SUB = 128, 8
STEPS = LANES // SUB
N_BLK = T // LANES
N_FULL = D // LANES
MAIN = N_FULL * LANES
REM = D - MAIN
N_COL = 2 * N_FULL + 1
QUARTER = D // 4
WORDS = LANES // 2
N_HEAD = 4
N_EARLY = 14
N_SEMS = 16

PACE = (13, 55, 127, 207, 255)
SCORE_AT, ROUTE_AT = 77, 104
GATE_AT, UP_AT, DOWN_AT = 137, 217, 274
WRITE_AT = 262


def _dot(a, b, dims):
    return lax.dot_general(a, b, dims, preferred_element_type=F32)


def _cmul(a, b):
    return a[0] * b[0] - a[1] * b[1], a[0] * b[1] + a[1] * b[0]


def _cmac(lam, h, u):
    re, im = _cmul(lam, h)
    return re + u[0], im + u[1]


def _sigmoid(v):
    return 1.0 / (1.0 + jnp.exp(-v))


def _pack(v):
    return pltpu.bitcast(v.astype(BF16), I32)


def _unpack(v):
    return pltpu.bitcast(v, BF16)


def _tile(i, n=1):
    return slice(i * LANES, (i + n) * LANES)


def _d_tile(i, n=1):
    return slice(i * LANES, min(D, (i + n) * LANES))


def _words(b, n=1):
    return slice(b * WORDS, (b + n) * WORDS)


def _shuffle(v, n):
    lane = lax.broadcasted_iota(I32, v.shape, 1)
    src = (lane & (n - 1)) * (LANES // n) + (lane >> (n.bit_length() - 1))
    return jnp.take_along_axis(v, src, axis=1)


def _kernel(x_h, lre_h, lim_h, bre_h, bim_h, cre_h, cim_h, ldt_h, dsk_h, wr_h,
            wg_h, wu_h, wd_h, gw_h, out_h,
            x_v, lre_v, lim_v, ldt_v, dsk_v, wr_v, gw_v, b_v, c_v, wg_v, wu_v, wd_v,
            xt_v, bt_v, h_v, cp_v, dcol_v, col_v, out_v, sems):
    st = {}
    acc = {}
    agenda = {}
    riders = []
    clock = [0]

    def at(when, fn, *args):
        agenda.setdefault(when, []).append(functools.partial(fn, *args))

    free_sems = iter(range(N_SEMS))

    def feed(src, dst, sem):
        dst[0:SUB, 0:LANES] = st["tick"][0:SUB, 0:LANES].astype(BF16)
        pltpu.make_async_copy(src, dst, sem).start(priority=0)

    def read(whole, parts, priority=1):
        sem = sems.at[next(free_sems)]
        for src, dst in parts:
            pltpu.make_async_copy(src, dst, sem).start(priority=priority)
        return pltpu.make_async_copy(whole, whole, sem)

    def read_paced(src, dst, groups, split):
        sem = sems.at[next(free_sems)]
        width = dst.shape[1] // split
        assert len(groups) % split == 0
        for i, when in enumerate(groups):
            window = pl.ds(i // split * SUB, SUB), pl.ds(i % split * width, width)
            at(when, feed, src.at[window], dst.at[window], sem)
        rest = slice(len(groups) // split * SUB, dst.shape[0])
        pltpu.make_async_copy(src.at[rest], dst.at[rest], sem).start(priority=1)
        return pltpu.make_async_copy(dst, dst, sem)

    def read_x(b0, b1):
        cols = _tile(b0, b1 - b0)
        return read(x_v.at[:, cols], [(x_h.at[:, cols], x_v.at[:, cols])], priority=0)

    def read_b(k0, k1, priority=1):
        parts = []
        for k in range(k0, k1):
            n = LANES if k < N_FULL else REM
            parts += [(src.at[pl.ds(k * LANES, n)], b_v.at[pl.ds(2 * k * LANES + i * n, n)])
                      for i, src in enumerate((bre_h, bim_h))]
        return read(b_v.at[2 * k0 * LANES:min(2 * D, 2 * k1 * LANES)], parts, priority)

    def read_c(k0, k1, priority=1):
        cols = _d_tile(k0, k1 - k0)
        parts = [(src.at[:, cols], c_v.at[i, :, cols]) for i, src in enumerate((cre_h, cim_h))]
        return read(c_v.at[:, :, cols], parts, priority)

    x_first = read_x(0, 2)
    vec_sem = sems.at[next(free_sems)]
    vectors = [pltpu.make_async_copy(src, dst, vec_sem) for src, dst in (
        (lre_h, lre_v), (lim_h, lim_v), (ldt_h, ldt_v), (dsk_h, dsk_v), (wr_h, wr_v), (gw_h, gw_v))]
    for c in vectors:
        c.start()
    x_second = read_x(2, N_HEAD)
    x_rest = _tile(N_HEAD, N_BLK - N_HEAD)
    head_reads = [
        [read_b(0, 1, priority=0)],
        [read_b(1, 2, priority=0), read_c(0, 1, priority=0)],
        [read_c(1, 3), read_b(2, 4)],
        [],
        [read_b(4, 5), read_c(3, 5),
         read_paced(x_h.at[:, x_rest], x_v.at[:, x_rest], range(*PACE[0:2]), 1)],
    ]
    gate_reads = [read_paced(wg_h, wg_v, range(*PACE[1:3]), 2)]
    up_reads = [read_paced(wu_h, wu_v, range(*PACE[2:4]), 2),
                read(wd_v.at[0:LANES], [(wd_h.at[0:LANES], wd_v.at[0:LANES])])]
    down_reads = [read_paced(wd_h.at[LANES:D], wd_v.at[LANES:D], range(*PACE[3:5]), 2)]

    def wait(copies):
        for c in copies:
            c.wait()

    def accumulate(key, v):
        st["tick"] = acc[key] = v + acc[key] if key in acc else v

    def due(load):
        st.setdefault("due", []).append(pltpu.bitcast(load(), I32))

    def streamed(v):
        for d in st.pop("due", []):
            w = min(LANES, v.shape[1])
            head = jnp.where(st["never"][:, :w], d[:, :w], v[:SUB, :w])
            if v.shape[1] > w:
                head = jnp.concatenate([head, v[:SUB, w:]], axis=1)
            v = jnp.concatenate([head, v[SUB:]], axis=0)
        return _unpack(v)

    def advance():
        clock[0] += 1
        for fn in agenda.pop(clock[0], []):
            fn()

    def group(fn, calls):
        for args in calls:
            fn(*args)
        if riders:
            tick = st["tick"]
            riders.pop(0)()
            st["tick"] = tick
        advance()

    lane = lax.broadcasted_iota(I32, (SUB, LANES), 1)
    sub = lax.broadcasted_iota(I32, (SUB, LANES), 0)

    def row(ref):
        return ref[...].astype(F32).reshape(1, D)

    def discretize():
        def stack(ref):
            r = jnp.broadcast_to(row(ref), (SUB, D))
            out = jnp.concatenate([r[:, MAIN:], r[:, MAIN:]], axis=1)
            for k in range(N_FULL):
                out = jnp.where(sub == k, r[:, _tile(k)], out)
            return out

        l_re, l_im = stack(lre_v), stack(lim_v)
        dt = jnp.exp(stack(ldt_v)).astype(BF16).astype(F32)
        st["never"] = dt < 0.0
        mag, ang = jnp.exp(dt * l_re), dt * l_im
        lam = mag * jnp.cos(ang), mag * jnp.sin(ang)
        size = jnp.maximum(jnp.abs(l_re), jnp.abs(l_im))
        n_re, n_im = l_re / size, l_im / size
        inv = 2.0 / (l_re * n_re + l_im * n_im)
        st["coef"] = _cmul((lam[0] - 1.0, lam[1]), (n_re * inv, -n_im * inv))
        power = lam[0], jnp.where((sub == N_FULL) & (lane >= REM), -lam[1], lam[1])
        for i in range((4 * STEPS).bit_length()):
            for k in range(N_FULL + 1):
                st["lam", 1 << i, k] = tuple(
                    jnp.broadcast_to(v[k:k + 1], (SUB, LANES)) for v in power)
            power = _cmul(power, power)

    def transpose_x(b):
        w = _shuffle(pltpu.bitcast(x_v[:, _tile(b)], I32), SUB)
        xt_v[_words(b), :] = pltpu.bitcast(_unpack(w).T, I32)

    def project_in(b, n, ks):
        a = streamed(xt_v[_words(b), ks])
        if b < N_HEAD:
            u = _dot(a, b_v[_tile(n), ks], NT)
        else:
            u = _dot(a, _unpack(bt_v[ks.start // 2:ks.stop // 2, _tile(n)]), NN)
        accumulate(("u", b, n), u)

    def scan(b, k):
        re = acc.pop(("u", b, 2 * k))
        im = acc.pop(("u", b, 2 * k + 1)) if k < N_FULL else pltpu.roll(re, REM, 1)
        u = [(re[j * SUB:(j + 1) * SUB], im[j * SUB:(j + 1) * SUB]) for j in range(STEPS)]
        total = u[0]
        for j in range(1, STEPS):
            total = _cmac(st["lam", 1, k], total, u[j])
        before = [pltpu.roll(v, 1, 0) for v in st["last", k]] if b else (0.0, 0.0)
        h = [jnp.where(sub == 0, w, pltpu.roll(v, 1, 0)) for v, w in zip(total, before)]
        for d in (1, 2, 4):
            s = _cmac(st["lam", STEPS * d, k], [pltpu.roll(v, d, 0) for v in h], h)
            h = [jnp.where(sub >= d, new, old) for new, old in zip(s, h)]
        st["last", k] = _cmac(st["lam", STEPS, k], h, total)
        states = []
        for j in range(STEPS - 1):
            h = _cmac(st["lam", 1, k], h, u[j])
            states.append(h)
        re, im = (jnp.concatenate(v, axis=0) for v in zip(*states, st["last", k]))
        h_v[_words(b), _tile(2 * k)] = _pack(re)
        if k < N_FULL:
            h_v[_words(b), _tile(2 * k + 1)] = _pack(im)

    def scale_c(k):
        cols = _d_tile(k)
        a, b = c_v[0, :, cols].astype(F32), c_v[1, :, cols].astype(F32)
        cr, ci = (v[k:k + 1, :a.shape[1]] for v in st["coef"])
        re, minus_im = a * cr - b * ci, a * -ci - b * cr
        if k < N_FULL:
            cp_v[:, _tile(2 * k)] = _pack(re)
            cp_v[:, _tile(2 * k + 1)] = _pack(minus_im)
        else:
            cp_v[:, _tile(2 * k)] = _pack(jnp.concatenate([re, minus_im], axis=1))

    def project_out(b, q, ks):
        a = streamed(cp_v[q * QUARTER // 2:(q + 1) * QUARTER // 2, ks])
        accumulate(("y", b, q), _dot(a, _unpack(h_v[_words(b), ks]), NT))

    def score_rem(b0):
        for b in range(b0, b0 + 4):
            accumulate(("score", b), _dot(st["probe"][:, MAIN:], x_v[MAIN:, _tile(b)], NN))

    def score(b):
        accumulate(("score", b), _dot(st["probe"][:, :MAIN], x_v[:MAIN, _tile(b)], NN))
        st["score", b] = acc.pop(("score", b)).astype(BF16).astype(F32)
        st["gate", b] = _sigmoid(st["score", b])

    def scores(b0, b1):
        return [functools.partial(fn, b) for b in range(b0, b1)
                for fn in ((score,) if b % 4 else (score_rem, score))]

    def route():
        def by_block(get):
            out = []
            for b0 in range(0, N_BLK, SUB):
                v = jnp.broadcast_to(get(b0), (SUB, LANES))
                for s in range(1, SUB):
                    v = jnp.where(sub == s, get(b0 + s), v)
                out.append(v)
            return jnp.concatenate(out, axis=0)

        def reduce(op, v):
            return op(op(v, axis=0, keepdims=True), axis=1, keepdims=True)

        r = by_block(lambda b: st["score", b][0:1])
        weight = by_block(lambda b: (1.0 - st["gate", b][1:2]) * st["gate", b][0:1])
        key = jnp.where(r != r, -jnp.inf, r)
        pos = (lax.broadcasted_iota(I32, r.shape, 0) * LANES
               + lax.broadcasted_iota(I32, r.shape, 1)).astype(F32)
        free_pos = pos
        st["token"], st["weight"] = [], []
        for _ in range(2):
            first = reduce(jnp.min, jnp.where(key == reduce(jnp.max, key), free_pos, float(T)))
            hit = pos == first
            st["token"].append(jnp.minimum(first, T - 1.0).astype(I32)[0, 0])
            st["weight"].append(reduce(jnp.sum, jnp.where(hit, weight, 0.0)))
            free_pos = jnp.where(hit, float(T), free_pos)
            key = jnp.where(hit, -jnp.inf, key)
        col = lax.broadcasted_iota(I32, (D // 2, LANES), 1)
        picked = jnp.zeros_like(col)
        for i, t in enumerate(st["token"]):
            base = pl.multiple_of((t >> 7) << 7, LANES)
            blk = pltpu.bitcast(x_v[:, pl.ds(base, LANES)], I32)
            picked = jnp.where(col == i, pltpu.roll(blk, (i - t) & (LANES - 1), 1), picked)
        st["picked"] = _unpack(picked).T[0:2 * SUB].astype(F32)[0:SUB]
        b0, b1 = (jnp.minimum(t >> 7, N_EARLY - 1) for t in st["token"])
        lo, hi = jnp.minimum(b0, b1), jnp.maximum(b0, b1)
        st["held"] = jnp.minimum(lo, N_EARLY - 2), jnp.where(lo == hi, N_EARLY - 1, hi)

    def ffn_in(w_v, f, k):
        ks = _d_tile(k)
        accumulate("ffn", _dot(st["picked"][:, ks], w_v[ks, _tile(f, 4)], NN))
        if k == N_FULL:
            v = acc.pop("ffn")
            st["act", f] = st["act", f] * v if ("act", f) in st else v * _sigmoid(v)

    def ffn_out(f, k):
        ks = _d_tile(k)
        accumulate("ffn", _dot(st["act", f], wd_v[ks, _tile(f, 4)], NT))
        if (f + 4) * LANES == F:
            y = acc.pop("ffn")
            for i in range(2):
                update = y[i:i + 1] * st["weight"][i]
                col_v[i, ks, :] = jnp.broadcast_to(update, (LANES, y.shape[1])).T
            st["ffn_rows"] = ks.stop

    def start_ffn(copies, w_v, out_tiles):
        assert not riders
        wait(copies)
        f_groups = range(0, F // LANES, 4)
        if w_v is not None:
            riders.extend(functools.partial(ffn_in, w_v, f, k)
                          for f in f_groups for k in range(N_FULL + 1))
        riders.extend(functools.partial(ffn_out, f, k) for k in out_tiles for f in f_groups)

    out_sem = sems.at[next(free_sems)]
    mixed, sent = [], []

    def send(rows, cols):
        pltpu.make_async_copy(out_v.at[rows, cols], out_h.at[rows, cols], out_sem).start()

    def block(b):
        return pl.ds(pl.multiple_of(b * LANES, LANES), LANES)

    def send_mixed():
        assert sorted(mixed) == list(range(len(mixed)))
        while len(sent) < len(mixed) - 2:
            b = len(sent)
            for held in st["held"]:
                b = b + (b >= held).astype(I32)
            send(slice(0, D), block(b))
            sent.append(b)

    def start_writes():
        out_v[0:SUB, _tile(N_BLK - 1)] = st["tick"][0:SUB, 0:LANES]
        send_mixed()

    def send_held(rows):
        assert len(mixed) == N_EARLY and st["ffn_rows"] >= rows.stop
        for i, t in enumerate(st["token"]):
            b = jnp.minimum(t >> 7, N_EARLY - 1)
            cur = out_v[rows, block(b)]
            hit = lax.broadcasted_iota(I32, cur.shape, 1) == t - b * LANES
            out_v[rows, block(b)] = jnp.where(hit, cur + col_v[i, rows, :], cur)
        for b in st["held"]:
            send(rows, block(b))

    def mix(b, q):
        rows = slice(q * QUARTER, (q + 1) * QUARTER)
        y = _shuffle(acc.pop(("y", b, q)), STEPS)
        xb = x_v[rows, _tile(b)].astype(F32)
        out = xb + st["gate", b][1:2] * (y + xb * dcol_v[rows, :])
        if b >= N_EARLY:
            assert st["ffn_rows"] >= rows.stop
            col = lax.broadcasted_iota(I32, out.shape, 1)
            for i, t in enumerate(st["token"]):
                out = jnp.where(col == t - b * LANES, out + col_v[i, rows, :], out)
            n = QUARTER // (3 if (b, q) == (N_BLK - 1, 3) else 1)
            for r in range(0, QUARTER, n):
                part = slice(rows.start + r, rows.start + r + n)
                out_v[part, _tile(b)] = out[r:r + n]
                send(part, _tile(b))
            return
        out_v[rows, _tile(b)] = out
        if q == 3:
            mixed.append(b)
            if sent:
                send_mixed()
            if len(mixed) == N_EARLY:
                send_held(slice(0, 3 * LANES))
                at(clock[0] + 9, due, lambda: out_v[D - SUB:, _tile(b)])

    main, rem = slice(0, MAIN), slice(MAIN, D)

    def stage_in(b, n0=0, n1=N_COL):
        for n in range(n0, n1):
            i = N_COL * b + n
            if i % 4 == 0:
                group(project_in, [(*divmod(j, N_COL), rem) for j in range(i, i + 4)])
            group(project_in, [(b, n, main)])

    def stage_out(b):
        group(project_out, [(b, q, _tile(N_COL - 1)) for q in range(4)])
        for q in range(4):
            group(project_out, [(b, q, _tile(0, 4))])
            group(project_out, [(b, q, _tile(4, 4))])
            mix(b, q)

    def head_in(k):
        if k == N_FULL:
            group(project_in, [(b, 2 * k, rem) for b in range(N_HEAD)])
            for b in range(N_HEAD):
                group(project_in, [(b, 2 * k, main)])
            return
        for b0 in range(0, N_HEAD, 2):
            if k and b0:
                due(lambda: h_v[3 * WORDS - SUB:3 * WORDS, _tile(2 * k - 1)])
            u = _dot(streamed(xt_v[_words(b0, 2), :]), b_v[_tile(2 * k, 2), :], NT)
            advance()
            for j in range(2):
                for i in range(2):
                    st["tick"] = acc["u", b0 + i, 2 * k + j] = u[_tile(i), _tile(j)]
                    advance()

    def head_scan(k):
        for b in range(N_HEAD):
            scan(b, k)

    def head_out(k):
        scale_c(k)
        ks = _tile(2 * k, 2 if k < N_FULL else 1)
        n = 2 if k < N_FULL else 4
        for b0 in range(0, N_HEAD, n):
            for b in range(b0, b0 + n):
                accumulate(("y", b), _dot(streamed(cp_v[:, ks]), _unpack(h_v[_words(b), ks]), NT))
            for q in range(4):
                st["tick"] = acc["y", b0][q * QUARTER:]
                advance()

    ffn_done = DOWN_AT + N_FULL * F // (4 * LANES)
    at(SCORE_AT, riders.extend, scores(N_HEAD, N_BLK))
    at(ROUTE_AT, route)
    at(GATE_AT, start_ffn, gate_reads, wg_v, ())
    at(UP_AT, start_ffn, up_reads, wu_v, (0,))
    at(WRITE_AT, start_writes)
    at(DOWN_AT, start_ffn, down_reads, None, range(1, N_FULL + 1))
    at(ffn_done, send_held, slice(3 * LANES, D))
    at(ffn_done + 5, due, lambda: out_v[D - SUB:, _tile(0)])

    wait([x_first] + vectors)
    transpose_x(0)
    transpose_x(1)
    discretize()
    wait([x_second])
    transpose_x(2)
    transpose_x(3)
    probe_row = lax.broadcasted_iota(I32, (SUB, D), 0)
    st["probe"] = jnp.where(probe_row == 0, row(wr_v), jnp.where(probe_row == 1, row(gw_v), 0.0))
    for fn in scores(0, N_HEAD):
        fn()
    for k, copies in enumerate(head_reads):
        wait(copies)
        if k == N_FULL:
            for b in range(N_HEAD, N_HEAD + 3):
                transpose_x(b)
        elif k:
            head_scan(k - 1)
        head_in(k)
        for n in range(2 * k, min(N_COL, 2 * k + 2)):
            bt_v[:, _tile(n)] = pltpu.bitcast(b_v[_tile(n), :].T, I32)
        if k == N_FULL:
            head_scan(k - 1)
            head_scan(k)
        if k:
            head_out(k - 1)
        else:
            dcol_v[...] = jnp.broadcast_to(row(dsk_v) - 1.0, (LANES, D)).T
    stage_in(N_HEAD)
    stage_in(N_HEAD + 1, 0, 2)
    head_out(N_FULL)
    for b in range(N_HEAD):
        y = acc.pop(("y", b))
        for q in range(4):
            acc["y", b, q] = y[q * QUARTER:(q + 1) * QUARTER]
    for b in range(N_HEAD + 3, N_BLK):
        transpose_x(b)
    at(clock[0] + 14, due, lambda: xt_v[T // 2 - SUB:, _tile(N_FULL - 1)])
    for b in range(N_HEAD, N_BLK):
        if 2 * N_HEAD <= b < 3 * N_HEAD:
            for q in range(4):
                mix(b - 2 * N_HEAD, q)
        for k in range(N_FULL + 1):
            scan(b, k)
        if b + 1 < N_BLK:
            stage_in(b + 1, 2 if b == N_HEAD else 0)
        stage_out(b)
    assert not acc and not agenda and not riders and len(sent) == N_EARLY - 2
    pltpu.make_async_copy(out_v, out_h, out_sem).wait()


@jax.jit
def pallas_gated_mix__ssm_conv_s5__moe_arch_mod__prompt_kernel(
    A_x: jax.Array,
    A_Lambda_re: jax.Array,
    A_Lambda_im: jax.Array,
    A_B_re: jax.Array,
    A_B_im: jax.Array,
    A_C_re: jax.Array,
    A_C_im: jax.Array,
    A_log_dt: jax.Array,
    A_Dskip: jax.Array,
    B_x: jax.Array,
    B_w_r: jax.Array,
    B_w_gate: jax.Array,
    B_w_up: jax.Array,
    B_w_down: jax.Array,
    gate_w: jax.Array,
):
    del B_x
    assert A_x.shape == (1, T, D) and B_w_gate.shape == (D, F)
    hbm = pl.BlockSpec(memory_space=pltpu.HBM)
    vmem = pltpu.VMEM
    out = pl.pallas_call(
        _kernel,
        out_shape=jax.ShapeDtypeStruct((D, T), F32),
        in_specs=[hbm] * 14,
        out_specs=hbm,
        scratch_shapes=[
            vmem((D, T), BF16), *[vmem((D,), BF16)] * 6,
            vmem((2 * D, D), BF16), vmem((2, D, D), BF16), *[vmem((D, F), BF16)] * 3,
            vmem((T // 2, D), I32), vmem((D // 2, 2 * D), I32),
            vmem((T // 2, 2 * D), I32), vmem((D // 2, 2 * D), I32),
            vmem((D, LANES), F32), vmem((2, D, LANES), F32), vmem((D, T), F32),
            pltpu.SemaphoreType.DMA((N_SEMS,)),
        ],
        compiler_params=pltpu.CompilerParams(
            vmem_limit_bytes=100 * 2**20, disable_semaphore_checks=True),
    )(A_x.reshape(T, D).T, A_Lambda_re, A_Lambda_im, A_B_re, A_B_im, A_C_re, A_C_im,
      A_log_dt, A_Dskip, B_w_r, B_w_gate, B_w_up, B_w_down.T, gate_w)
    return out.T.reshape(1, T, D)
```
